```python
import os as _os
_os.environ.setdefault('JAX_PLATFORMS', 'cpu')
import jax
import jax.numpy as jnp

def _softmax(x, axis=-1):
    return jax.nn.softmax(x, axis=axis)

def _gelu(x):
    return jax.nn.gelu(x, approximate=True)

def _silu(x):
    return jax.nn.silu(x)

def _sigmoid(x):
    return jax.nn.sigmoid(x)

def _layernorm(x, axis=-1, eps=1e-05):
    m = jnp.mean(x, axis=axis, keepdims=True)
    v = jnp.var(x, axis=axis, keepdims=True)
    return (x - m) / jnp.sqrt(v + eps)

def _scatter_add(tgt, idx, src, axis=0):
    return tgt.at[idx].add(src)

def _segment_sum(src, seg, n):
    return jax.ops.segment_sum(src, seg, n)

class _Rng:

    def __init__(self, key):
        self._k = key

    def _next(self):
        self._k, sub = jax.random.split(self._k)
        return sub

    def normal(self, shape):
        return jax.random.normal(self._next(), shape, dtype=jnp.bfloat16)

    def randint(self, lo, hi, shape):
        return jax.random.randint(self._next(), shape, lo, hi, dtype=jnp.int32)

    def uniform(self, shape, lo=0.0, hi=1.0):
        return jax.random.uniform(self._next(), shape, jnp.bfloat16, lo, hi)

    def permutation(self, n):
        return jax.random.permutation(self._next(), n)
kernel_name = 'interleave_layers__memory_aug_recurrent_mem_tr__mixer_token_mlp__prompt'

def setup_inputs():
    _rng = _Rng(jax.random.key(int.from_bytes(__import__("os").urandom(4), "little")))
    _w = lambda a: (lambda t: t.astype(jnp.bfloat16) if jnp.issubdtype(t.dtype, jnp.floating) else t)(jnp.asarray(a))

    def _A_setup():
        B, S, Dm = (1, 2048, 640)
        H, Dh = (32, 128)
        M, seg = (8, 32)
        seg = min(seg, S)
        S = S // seg * seg
        return {'x': _w((lambda *s: _rng.normal(s) * 0.05)(B, S, Dm)), 'mem0': _w((lambda *s: _rng.normal(s) * 0.2)(B, M, Dm)), 'Wq': _w((lambda *s: _rng.normal(s) * 0.8)(Dm, H, Dh) * Dm ** (-0.5)), 'Wk': _w((lambda *s: _rng.normal(s) * 0.8)(Dm, H, Dh) * Dm ** (-0.5)), 'Wv': _w((lambda *s: _rng.normal(s) * 0.2)(Dm, H, Dh) * Dm ** (-0.5)), 'Wo': _w((lambda *s: _rng.normal(s) * 0.2)(H, Dh, Dm) * (H * Dh) ** (-0.5)), 'seg_len': seg}
    _A_in = _A_setup()

    def _B_setup():
        B, S, D, F = (1, 2048, 640, 1728)
        return {'x': _w((lambda *s: _rng.normal(s) * 0.05)(B, S, D)), 'w1': _w((lambda *s: _rng.normal(s) * 0.2)(S, F) * S ** (-0.5)), 'b1': _w((lambda *s: _rng.normal(s) * 0.2)(F) * 0.02), 'w2': _w((lambda *s: _rng.normal(s) * 0.2)(F, S) * F ** (-0.5)), 'b2': _w((lambda *s: _rng.normal(s) * 0.2)(S) * 0.02)}
    _B_in = _B_setup()
    return {'A_x': _A_in['x'], 'A_mem0': _A_in['mem0'], 'A_Wq': _A_in['Wq'], 'A_Wk': _A_in['Wk'], 'A_Wv': _A_in['Wv'], 'A_Wo': _A_in['Wo'], 'A_seg_len': _A_in['seg_len'], 'B_x': _B_in['x'], 'B_w1': _B_in['w1'], 'B_b1': _B_in['b1'], 'B_w2': _B_in['w2'], 'B_b2': _B_in['b2']}

def reference(A_x, A_mem0, A_Wq, A_Wk, A_Wv, A_Wo, A_seg_len, B_x, B_w1, B_b1, B_w2, B_b2):

    def _A_ref(x, mem0, Wq, Wk, Wv, Wo, seg_len):
        B, S, Dm = x.shape
        H, Dh = (Wq.shape[1], Wq.shape[2])
        M = mem0.shape[1]
        scale = Dh ** (-0.5)
        n_seg = S // seg_len
        L = M + seg_len
        idx = jnp.arange(L)
        mask = (idx[:, None] < M) | (idx[:, None] >= idx[None, :])
        mem = mem0
        outs = []
        for s in range(n_seg):
            xs = x[:, s * seg_len:(s + 1) * seg_len, :].copy()
            h = jnp.concatenate([mem, xs], axis=1)
            q = jnp.einsum('btd,dhe->bhte', h, Wq)
            k = jnp.einsum('btd,dhe->bhte', h, Wk)
            v = jnp.einsum('btd,dhe->bhte', h, Wv)
            scores = jnp.einsum('bhqe,bhke->bhqk', q, k) * scale
            scores = jnp.where(mask[None, None], scores, -1000000000.0)
            p = _softmax(scores, axis=-1)
            o = jnp.einsum('bhqk,bhke->bhqe', p, v)
            o = jnp.einsum('bhte,hed->btd', o, Wo)
            mem = o[:, :M, :].copy()
            outs.append(o[:, M:, :])
        return jnp.concatenate(outs, axis=1)

    def _B_ref(x, w1, b1, w2, b2):
        B, S, D = x.shape
        h = _layernorm(x, axis=-1)
        u = jnp.einsum('bsd,sf->bdf', h, w1) + b1
        u = _gelu(u)
        y = jnp.einsum('bdf,fs->bds', u, w2) + b2
        return (lambda x, *d: x.transpose(*d))(y, 0, 2, 1)
    x = A_x
    x = x + _A_ref(_layernorm(x, axis=-1), A_mem0, A_Wq, A_Wk, A_Wv, A_Wo, A_seg_len)
    x = x + _B_ref(_layernorm(x, axis=-1), B_w1, B_b1, B_w2, B_b2)
    x = x + _A_ref(_layernorm(x, axis=-1), A_mem0, A_Wq, A_Wk, A_Wv, A_Wo, A_seg_len)
    x = x + _B_ref(_layernorm(x, axis=-1), B_w1, B_b1, B_w2, B_b2)
    return x
```

```python
import contextlib
import functools
import math

import numpy as np
import jax
import jax.numpy as jnp
from jax import lax
import jax.experimental.pallas as pl
import jax.experimental.pallas.tpu as pltpu

F32 = jnp.float32
BF16 = jnp.bfloat16
U32 = jnp.uint32
EPS = 1e-5
LOG2E = math.log2(math.e)
T = 128
TP = T // 2

NN = (((1,), (0,)), ((), ()))
NT = (((1,), (1,)), ((), ()))

CFG = dict(
    n_pro=12,
    d_qs=280,
    d_sp=600,
    d_gap=0,
    op_group=2,
    op_last=8,
    post_u=1,
    pre_u=2,
    mix_bf16=True,
    up_group=2,
    only=None,
)


def _terms(b, prod):
    kind, i, j = prod
    if kind < 3:
        return ((((1, i, 1), (1, j, 0)), ((1, i, 0), (1, j, 1))),
                (((1, i, 0), (-1, j, 0)), ((1, i, 0), (1, j, 0))),
                (((1, j, 1), (-1, i, 1)), ((1, i, 1), (1, j, 1))))[kind]
    h = int(i >= b)
    return ((((1, i, 0), (1, i, 1)), ((1, i, h),)),
            (((1, i, 1 - h),), ((1, i, 1 - h), (-1, i, h))))[kind - 3]


def _edge(i, j):
    return [(kind, i, j) for kind in range(3)]


def _corners(v):
    return [(3, v, v), (4, v, v)]


def _scheme_diagonal(b):
    prods = []
    for m in range(b):
        prods += [p for j in range(b) if j != m for p in _edge(m, b + j)]
        prods += _edge(m, b + m) + _corners(m) + _corners(b + m)
    return prods


def _scheme_blocked(b):
    prods = []
    for n, j0 in enumerate(range(b, 2 * b, 2)):
        for i in range(b):
            prods += _edge(i, j0) + _edge(i, j0 + 1) + [_corners(i)[n], _corners(j0 + i // 2)[i % 2]]
    return prods


def _scheme_nested(b):
    prods = []
    for m in range(b):
        prods += _corners(m) + [p for j in range(m) for p in _edge(m, b + j)]
        prods += _corners(b + m) + [p for i in range(m + 1) for p in _edge(i, b + m)]
    return prods


def _scheme_grouped():
    b = 7
    corners = {v: _corners(v) for v in range(2 * b)}

    def square(i, j):
        return [[(kind, i + x, b + j + y) for x in range(2) for y in range(2)] for kind in range(3)]

    def single(i, j, *owners):
        return [_edge(i, b + j) + [corners[v].pop(0) for v in owners]]

    groups = []
    for m in range(1, b):
        groups += single(0, m, b + m) + single(m, 0, m)
    groups += single(0, 0, 0, 0) + [corners.pop(b)]
    groups += square(1, 3) + square(3, 1) + square(1, 5) + square(5, 1)
    groups += single(1, 2, b + 2) + single(2, 1, b + 1) + single(1, 1, 1) + single(2, 2, 2)
    groups += square(3, 5)
    groups += single(5, 3) + single(6, 3) + single(3, 4) + single(4, 3) + single(3, 3, 3, b + 3)
    groups += single(5, 4) + single(6, 4) + single(4, 4, 4, b + 4)
    groups += single(5, 6) + single(6, 5) + single(5, 5, 5, b + 5) + single(6, 6, 6, b + 6)
    return groups


def _weights(b, fold_inputs, tile):
    @functools.cache
    def link(u, v):
        m, n = u % b, v % b
        others = [k for k in range(b) if k != m]
        if m != n:
            if fold_inputs:
                return (1, tile(m, v))
            return (1 if u >= b else -1, tile(u, n))
        if fold_inputs:
            if u >= b:
                return (1, tile(b, v)) if v >= b else _signed_sum(
                    [(1, tile(b, m))] + [(-1, tile(k, m)) for k in others])
            if v >= b:
                return _sadd((1, tile(m, v)), (-1, tile(b, v)))
            return _sadd((1, tile(m, m)), _neg(link(b + m, m)))
        if u >= b:
            return (1, tile(u, b)) if v >= b else _sadd((1, tile(u, m)), (1, tile(u, b)))
        if v >= b:
            return _signed_sum([(1, tile(m, b))] + [(1, tile(m, k)) for k in others])
        return _sadd((1, tile(m, m)), link(m, b + m))

    def weight(prod):
        kind, i, j = prod
        if kind == 0:
            return _sadd(link(i, j), link(j, i))
        if kind < 3:
            return link(i, j) if kind == 1 else link(j, i)
        across = range(b) if i >= b else range(b, 2 * b)
        if kind == 3:
            if fold_inputs:
                return _signed_sum([link(i, i)] + [_neg(link(i, w)) for w in across])
            if i < b:
                return _sadd(link(i, i), (-1, tile(i, b)))
            return _signed_sum((-1, tile(i, k)) for k in range(b))
        if not fold_inputs:
            return _signed_sum([link(i, i)] + [link(w, i) for w in across])
        if i < b:
            return _sadd(link(i, i), (1, tile(b, i)))
        return _signed_sum((1, tile(k, i)) for k in range(b))
    return weight


def _is_plain(b, prod):
    kind, i, j = prod
    return kind in (1, 2) and i != j - b


QKV_FIRST, QKV, OUT, MIX = _scheme_diagonal(4), _scheme_blocked(4), _scheme_nested(4), _scheme_grouped()
SLOT = {p: n for n, p in enumerate(p for p in QKV if not _is_plain(4, p))}


def _neg(a):
    return (-a[0], a[1])


def _sadd(a, b):
    if a is None:
        return b
    if a[0] == b[0]:
        return (a[0], a[1] + b[1])
    return (1, a[1] - b[1]) if a[0] > 0 else (1, b[1] - a[1])


def _sval(a):
    return a[1] if a[0] > 0 else -a[1]


def _signed_sum(terms):
    acc = None
    for t in terms:
        acc = _sadd(acc, t)
    return acc


def _operand(b, prod, block):
    return _signed_sum((s, block(v, h)) for s, v, h in _terms(b, prod)[0])


def _scatter(b, acc, results):
    update = {}
    for prod, sign, value in results:
        for s, v, h in _terms(b, prod)[1]:
            update[v, h] = _sadd(update.get((v, h)), (s * sign, value))
    for key, term in update.items():
        acc[key] = _sadd(acc.get(key), term)


def _folded_inputs(b, block):
    return lambda v, h: block(v, h) if v < b else block(b, h) + block(v - b, h)


def _folded_output(acc, b, n, h):
    if n < b:
        return _sadd(acc[n, h], _neg(acc[b + n, h]))
    return _signed_sum(acc[b + j, h] for j in range(b))


def _dot(a, b, dims=NN):
    return lax.dot_general(a, b, dims, preferred_element_type=F32)


def _layernorm(x):
    inv_d = 1.0 / x.shape[-1]
    m = jnp.sum(x, axis=-1, keepdims=True) * inv_d
    c = x - m
    v = jnp.sum(c * c, axis=-1, keepdims=True) * inv_d
    return c * lax.rsqrt(v + EPS)


def _gelu(x):
    k = math.sqrt(2.0 / math.pi)
    inner = x * (k + (k * 0.044715) * (x * x))
    hx = 0.5 * x
    return hx + hx * jnp.tanh(inner)


def _unpacked(x):
    return pltpu.bitcast(x, BF16)


def _packed(x):
    return pltpu.bitcast(x.astype(BF16), U32)


def _low(x):
    return pltpu.bitcast(x << 16, F32)


def _high(x):
    return pltpu.bitcast(x & jnp.uint32(0xFFFF0000), F32)


def _split_rows(words):
    return jnp.concatenate([_low(words), _high(words)], axis=0)


def _join_rows(v):
    v = pltpu.bitcast(v.astype(BF16).astype(F32), U32)
    n = v.shape[0] // 2
    return (v[0:n] >> 16) | v[n:]


def _ds(start, size, align=None):
    if isinstance(start, int):
        return pl.ds(start, size)
    return pl.ds(pl.multiple_of(start, align or size), size)


def _kernel(x_hbm, mem0_ref, wq_hbm, wk_hbm, wv_hbm, wo_hbm, w1t_hbm, b1_ref, w2_hbm, b2_ref,
            out_hbm,
            xio, xpro, pro_lhs, mem, od, hn, xn0, raw, wqkv, wqkv_hk, wo, wo_hk, wmix,
            lhs, act, o_main, o_x, x_sem, w_sem, wo_sem, mix_sem, out_sem,
            *, d_ff, cfg):
    n_seg, seg, D = x_hbm.shape
    S = n_seg * seg
    M = mem0_ref.shape[0]
    L = M + seg
    H, E = wqkv.shape[1] * wqkv.shape[2], wqkv.shape[4]
    KT = D // T
    R = 32
    X = L - R
    P = R // X
    PR = seg * P
    XN = 2 * R - M
    n_per = n_seg // P
    n_pro = cfg["n_pro"]
    scale = float(E) ** -0.5
    assert (KT, E, X, P, PR, S // T, H) == (5, T, 8, 4, T, 16, 32)
    assert 13 * T < d_ff <= 14 * T and d_ff % 16 == 0 and n_pro % 2 == 0

    def spare_rows(j, i, h, r0=0, rn=R):
        return _ds((((j + 1) * 3 + i) * H + h) * R + r0, rn, X)

    def ht_rows(j, r0, rn):
        return _ds(j * 2 * D + r0, rn, X)

    def xs_rows(j, k, r0, rn):
        return _ds(j * 2 * D + D + k * T + r0, rn, X)

    def scope(n):
        return jax.named_scope(n) if cfg.get('scopes') else contextlib.nullcontext()

    cp_xpro = pltpu.make_async_copy(x_hbm.at[0:n_pro * P, R - M:seg, :], xpro, x_sem.at[n_per])

    def cp_x(j):
        segs = pl.ds(j * P, P)
        return pltpu.make_async_copy(x_hbm.at[segs], xio.at[segs], x_sem.at[j])

    def cp_w(w, c, g):
        return [pltpu.make_async_copy(w.bitcast(U32).at[:, p, g],
                                      raw.at[pl.ds(c * (D // 2), D // 2), pl.ds(4 * p, 4), :], w_sem.at[c])
                for p in range(2)]

    def cp_wo(g):
        return [pltpu.make_async_copy(wo_hbm.bitcast(U32).at[:, g, :, n * T:(n + 1) * T],
                                      wo.at[n, :, g], wo_sem.at[g]) for n in range(KT)]

    def start_chunk(c, g, i):
        for n, w in enumerate((wq_hbm, wk_hbm, wv_hbm)):
            @pl.when(i == n)
            def _():
                for cp in cp_w(w, c, g):
                    cp.start()

        @pl.when(i == 2)
        def _():
            for cp in cp_wo(g):
                cp.start()

    cp_mix = [pltpu.make_async_copy(w.bitcast(U32).at[:, t * T:(t + 1) * T],
                                    wmix.at[i, t, 0:d_ff // 2, :], mix_sem.at[i])
              for i, w in enumerate((w1t_hbm, w2_hbm)) for t in range(S // T)]

    with scope('pro_issue'):
        cp_xpro.start()
        for cp in cp_w(wq_hbm, 0, 0):
            cp.start()

    wmix[:, :, d_ff // 2:, :] = jnp.zeros((2, S // T, wmix.shape[2] - d_ff // 2, T), U32)
    with scope('pro_wait'):
        cp_xpro.wait()
        for cp in cp_w(wk_hbm, 1, 0):
            cp.start()
    xn = _layernorm(xpro[...].astype(F32).reshape(n_pro * R, D))
    hp = n_pro * R // 2
    block = _folded_inputs(4, lambda k, h: xn[h * hp:(h + 1) * hp, k * T:(k + 1) * T])
    qkv_sign, out_sign = {}, {}
    for r, prod in enumerate(QKV_FIRST):
        qkv_sign[prod], v = _operand(4, prod, block)
        pro_lhs[r] = _packed(v)

    def prologue(c, carry):
        g = c // 3
        i = c - 3 * g

        @pl.when(c == 0)
        def _():
            start_chunk(2, 0, c + 2)

        @pl.when(g < 3)
        def _():
            start_chunk(c + 3, g + 1, i)

        @pl.when(c == 10)
        def _():
            cp_x(0).start()
            cp_x(1).start()

        for cp in cp_w(wq_hbm, c, 0):
            cp.wait()
        source = raw.reshape(raw.shape[0] * 8, E)
        ready = set()

        def words(k, h):
            if (k, h // 2) not in ready:
                ready.add((k, h // 2))
                row = (c * (D // 2) + k * TP) * 8 + h // 2
                even, odd = [source[pl.ds(row + 4 * p, TP, stride=8), :] for p in range(2)]
                wqkv[i, g, h // 2 * 2, k * TP:(k + 1) * TP, :] = (even & jnp.uint32(0xFFFF)) | (odd << 16)
                wqkv[i, g, h // 2 * 2 + 1, k * TP:(k + 1) * TP, :] = (even >> 16) | (odd & jnp.uint32(0xFFFF0000))
            return wqkv[i, g, h, k * TP:(k + 1) * TP, :]

        plain = _weights(4, True, words)
        combined = _weights(4, True, lambda k, h: _split_rows(words(k, h)))
        acc, group = {}, []
        for r, prod in enumerate(QKV_FIRST):
            if prod in SLOT:
                s, w = combined(prod)
                w = _join_rows(w)
                wqkv_hk[i, g, SLOT[prod]] = w
            else:
                s, w = plain(prod)
            qkv_sign[prod] *= s
            group.append((prod, qkv_sign[prod], _dot(_unpacked(pro_lhs[r]), _unpacked(w))))
            if len(group) == 4:
                _scatter(4, acc, group)
                group = []
        for h in range(8):
            for half in range(2):
                v = _sval(acc[h, half])
                for p in range(n_pro // 2):
                    act[spare_rows(half * (n_pro // 2) + p, i, 8 * g + h), :] = v[p * R:(p + 1) * R]

        @pl.when(i == 2)
        def _():
            for cp in cp_wo(g):
                cp.wait()

            combined = _weights(4, False, lambda v, n: _split_rows(wo[n, 2 * (v % 4) + v // 4, g]))
            for prod in QKV_FIRST:
                if prod in SLOT:
                    out_sign[prod], w = combined(prod)
                    wo_hk[SLOT[prod], g] = _join_rows(w)
        return carry

    if cfg["only"] is None or "pro" in cfg["only"]:
        with scope("prologue"):
            lax.fori_loop(0, 12, prologue, 0)
            cp_x(0).wait()

    qi = lax.broadcasted_iota(jnp.int32, (L, L), 0)
    ki = lax.broadcasted_iota(jnp.int32, (L, L), 1)

    def residual(j):
        for u in range(P):
            v = xio[j * P + u].astype(F32) + od[u * seg:(u + 1) * seg, :]
            for k in range(KT):
                act[xs_rows(j, k, u * seg, seg), :] = v[:, k * T:(k + 1) * T]

    def mix_input(j):
        for r in range(0, PR, 16):
            v = jnp.concatenate([act[xs_rows(j, k, r, 16), :] for k in range(KT)], axis=1)
            hn[r:r + 16, :] = _layernorm(_layernorm(v))
        for k in range(KT):
            act[ht_rows(j, k * T, T), :] = hn[:, k * T:(k + 1) * T].T

    def first_rows(j):
        xn0[0:R - M, :] = _layernorm(xio[j * P].astype(F32)[0:R - M])
        for u in range(P):
            xn0[R - M + u * X:R - M + (u + 1) * X, :] = _layernorm(xio[j * P + u].astype(F32)[R - M:seg])

    def period(j, carry, projected):
        if projected:
            cp_x(j + 1).wait()
            cp_x(j + 2).start()

            @pl.when(j == n_pro - 1)
            def _():
                for jj in range(n_pro + 2, n_per):
                    cp_x(jj).start()

            for i in range(4):
                @pl.when(j == i)
                def _():
                    for cp in cp_mix[8 * i:8 * i + 8]:
                        cp.start()
        mask = (qi < M) | (qi >= ki)
        prev = jnp.maximum(j - 1, 0)
        first = xn0[...]
        clock = [0]
        slot = j if projected else n_pro - 1
        mem_v = mem[...]
        residual(prev)
        for u in range(P):
            last = u == P - 1
            if u == cfg["post_u"]:
                mix_input(prev)
            if u == cfg["pre_u"]:
                first_rows(jnp.minimum(j + 1, n_per - 1))
            tok = first[0:R - M] if u == 0 else _layernorm(xio[j * P + u].astype(F32)[0:R - M])
            hs = jnp.concatenate([mem_v, tok], axis=0)
            qkv, prob, t_qk, t_s, t_p = {}, {}, {}, {}, {}
            nxt = dict(s=0, p=0, t=-1000)

            def full(h, i):
                return jnp.concatenate([qkv[h, i], act[spare_rows(slot, i, h, u * X, X), :]], axis=0)

            def scores(h):
                t = _dot(full(h, 0), full(h, 1).astype(BF16), NT) * (scale * LOG2E)
                t = jnp.where(mask, t, -1e9 * LOG2E)
                e = jnp.exp2(t - jnp.max(t, axis=-1, keepdims=True))
                l = jnp.sum(e, axis=-1, keepdims=True)
                r0 = pl.reciprocal(l, approx=True)
                prob[h] = e * (r0 * (2.0 - l * r0))

            def pv(h):
                o = _dot(prob[h], full(h, 2).astype(BF16))
                if last:
                    o_main[:, h * E:(h + 1) * E] = o[0:R]
                else:
                    o_main[0:R // 2, h * E:(h + 1) * E] = pltpu.bitcast(_packed(o[0:R]), F32)
                o_x[u * X:(u + 1) * X, h * E:(h + 1) * E] = o[R:L]

            t_v = {}

            def tick(tiles, rows=R, force=False):
                clock[0] += tiles * rows // 4
                while force or clock[0] >= nxt["t"] + cfg["d_gap"]:
                    h = nxt["p"]
                    if h in t_s and h in t_v and (
                            force or clock[0] >= max(t_s[h] + cfg["d_sp"], t_v[h] + cfg["d_qs"])):
                        pv(h)
                        t_p[h] = clock[0]
                        nxt["p"] += 1
                    elif nxt["s"] in t_qk and (force or clock[0] >= t_qk[nxt["s"]] + cfg["d_qs"]):
                        scores(nxt["s"])
                        t_s[nxt["s"]] = clock[0]
                        nxt["s"] += 1
                    else:
                        break
                    clock[0] += L // 4
                    nxt["t"] = clock[0]
                    force = False

            def need(h):
                while h not in t_p:
                    tick(0, force=True)

            stack = contextlib.ExitStack()
            if f'p{u}' in cfg.get('fine', ()):
                stack.enter_context(jax.named_scope(f'steps_proj{u}'))
            if u == 0 and not projected:
                rows = (hs, first[R - M:XN])
                block = _folded_inputs(4, lambda k, h: rows[h][:, k * T:(k + 1) * T])
                for r, prod in enumerate(QKV):
                    lhs[r] = _packed(_operand(4, prod, block)[1])
                for g in range(H // 8):
                    for i in range(3):
                        plain = _weights(4, True, lambda k, h: wqkv[i, g, h, k * TP:(k + 1) * TP, :])
                        acc = {}
                        for r, prod in enumerate(QKV):
                            w = wqkv_hk[i, g, SLOT[prod]] if prod in SLOT else plain(prod)[1]
                            _scatter(4, acc, [(prod, qkv_sign[prod], _dot(_unpacked(lhs[r]), _unpacked(w)))])
                            tick(1)
                        for h in range(8):
                            qkv[8 * g + h, i] = _sval(acc[h, 0])
                            act[spare_rows(slot, i, 8 * g + h), :] = _sval(acc[h, 1])
                            if i > 0:
                                (t_qk, t_v)[i - 1][8 * g + h] = clock[0]
            else:
                hs = hs.astype(BF16)
                for k in range(KT):
                    for h in range(2):
                        for i in range(3):
                            r = _dot(hs[:, k * T:(k + 1) * T], _unpacked(wqkv[i, 0, h, k * TP:(k + 1) * TP, :]))
                            qkv[h, i] = r if k == 0 else qkv[h, i] + r
                tick(6 * KT)
                t_qk[0] = t_qk[1] = t_v[0] = t_v[1] = clock[0]
                for h in range(2, H):
                    for i in range(3):
                        qkv[h, i] = _dot(hs, _unpacked(wqkv[i, h // 8, h % 8]))
                        if i > 0:
                            (t_qk, t_v)[i - 1][h] = clock[0] + KT * R // 4
                        tick(KT)

            stack.close()
            if f'o{u}' in cfg.get('fine', ()):
                stack.enter_context(jax.named_scope(f'steps_out{u}'))
            if last:
                acc = {}
                plain = _weights(4, False, lambda v, n: wo[n, 2 * (v % 4) + v // 4])
                for prod in OUT:
                    need(max(2 * (v % 4) + v // 4 for v in prod[1:]) * 4 + 3)

                    def heads(v, half):
                        c = (2 * (v % 4) + v // 4) * 4 * E
                        return (o_main, o_x)[half][:, c:c + 4 * E]
                    s, v = _operand(4, prod, heads)
                    sw, w = (out_sign.get(prod, 1), wo_hk[SLOT[prod]]) if prod in SLOT else plain(prod)
                    _scatter(4, acc, [(prod, s * sw, _dot(v.astype(BF16), _unpacked(w.reshape(4 * TP, T))))])
                    tick(4)
                o, ox = [jnp.concatenate([_sval(_folded_output(acc, 4, n, half)) for n in range(KT)], axis=1)
                         for half in range(2)]
                for uu in range(P):
                    od[uu * seg + R - M:(uu + 1) * seg, :] = ox[uu * X:(uu + 1) * X]
            else:
                acc = [None] * KT
                tail = H - cfg["op_last"]
                bounds = list(range(0, tail, cfg["op_group"])) + [tail, H]
                for h0, h1 in zip(bounds[:-1], bounds[1:]):
                    need(h1 - 1)
                    a = _unpacked(o_main[0:R // 2, h0 * E:h1 * E])
                    for n in range(KT):
                        w = jnp.concatenate([wo[n, h // 4, h % 4] for h in range(h0, h1)], axis=0)
                        r = _dot(a, _unpacked(w))
                        acc[n] = r if acc[n] is None else acc[n] + r
                        tick(h1 - h0)
                o = jnp.concatenate(acc, axis=1)
            stack.close()
            mem_v = o[0:M]
            od[u * seg:u * seg + R - M, :] = o[M:R]
        mem[...] = mem_v
        return carry

    def cp_out(j):
        segs = pl.ds(j * P, P)
        return pltpu.make_async_copy(xio.at[segs], out_hbm.at[segs], out_sem.at[j])

    def token_mix():
        half = D // 2
        b1 = b1_ref[...].astype(F32).reshape(1, d_ff)
        b1 = jnp.concatenate([b1, jnp.zeros((1, 14 * T - d_ff), F32)], axis=1)
        b2 = b2_ref[...].astype(F32).reshape(1, S)

        def run(fold_inputs, block, tile, dims, size, finish):
            plain = _weights(7, fold_inputs, tile)
            combined = _weights(7, fold_inputs, lambda u, v: tile(u, v).astype(F32))
            acc = {}
            for n, group in enumerate(MIX):
                for r in range(0, len(group), size):
                    results = []
                    for prod in group[r:r + size]:
                        s, v = _operand(7, prod, block)
                        sw, w = (plain if _is_plain(7, prod) else combined)(prod)
                        results.append((prod, s * sw, _dot(v.astype(BF16) if cfg["mix_bf16"] else v, w, dims)))
                    _scatter(7, acc, results)
                later = {v % 7 for grp in MIX[n + 1:] for prod in grp for v in prod[1:]}
                for m in sorted({v % 7 for prod in group for v in prod[1:]} - later):
                    finish(acc, m)
            return acc

        def w_tile(i, f, t):
            return _unpacked(wmix[i, t, f * TP:(f + 1) * TP, :])

        hidden = {}

        def activate(acc, m):
            for f in (m, 7 + m):
                for h in range(2):
                    hidden[f, h] = _gelu(_sval(_sadd(acc[f, h], (1, b1[:, f * T:(f + 1) * T]))))

        tokens = _folded_inputs(7, lambda n, h: jnp.concatenate(
            [act[ht_rows(2 * n + t, h * half, half), :] for t in range(2)], axis=1))
        run(True, tokens, lambda n, f: jnp.concatenate([w_tile(0, f, 2 * n + t) for t in range(2)], axis=1),
            NT, cfg["up_group"], activate)

        for t in range(2):
            def emit(acc, n):
                j = 2 * n + t
                y = jnp.concatenate([_sval(_sadd(_folded_output(acc, 7, n, h), (1, b2[:, j * T:(j + 1) * T])))
                                     for h in range(2)], axis=0)
                v = jnp.concatenate([act[xs_rows(j, k, 0, T), :] for k in range(KT)], axis=1) + y.T
                xio[j * P:(j + 1) * P] = v.reshape(P, seg, D).astype(BF16)
                cp_out(j).start()
            emit(run(False, lambda f, h: hidden[f, h], lambda f, n: w_tile(1, f, 2 * n + t), NN, 4, emit), 7)

    def layer(li, carry):
        mem[...] = mem0_ref[...].astype(F32)
        od[...] = jnp.zeros(od.shape, F32)
        first_rows(0)
        n_first = jnp.where(li == 0, n_pro, 0)
        if cfg.get("skip_a"):
            n_first = 0

            @pl.when(li == 0)
            def _():
                for jj in range(2, n_per):
                    cp_x(jj).start()
                for cp in cp_mix:
                    cp.start()
                for jj in range(1, n_pro + 1):
                    cp_x(jj).wait()
        elif cfg["only"] is None or "a" in cfg["only"]:
            with scope('steps_a'):
                lax.fori_loop(0, n_first, functools.partial(period, projected=True), 0)

        @pl.when(li == 0)
        def _():
            for j in range(n_pro + 1, n_per):
                cp_x(j).wait()
            for cp in cp_mix:
                cp.wait()
        if cfg["only"] is None or "b" in cfg["only"]:
            with scope('steps_b'):
                lax.fori_loop(n_first, n_per, functools.partial(period, projected=False), 0)

        @pl.when(li > 0)
        def _():
            for j in range(n_per):
                cp_out(j).wait()
        if cfg.get("skip_mix"):
            xio[0, :, 0:T] = (act[pl.ds(pl.multiple_of(li * 8, 8), 32), :] + od[0:32, 0:T]).astype(BF16)
            for j in range(n_per):
                cp_out(j).start()
        elif cfg["only"] is None or "mix" in cfg["only"]:
            with scope('mix'):
                residual(n_per - 1)
                mix_input(n_per - 1)
                token_mix()
        if cfg["only"] is not None:
            z = pl.multiple_of(li * 8, 8)
            v = wqkv_hk[li, li, li, pl.ds(z, 32), :] + wo_hk[li, li, pl.ds(z, 32), :] + wqkv[li, li, li, pl.ds(z, 32), :]
            v = pltpu.bitcast(v, F32) + act[pl.ds(z, 32), :] + od[pl.ds(z, 32), 0:T]
            xio[li, :, 0:T] = v.astype(BF16)
            cp_out(0).start()
        return carry

    with scope('layers'):
        lax.fori_loop(0, 2, layer, 0)
    for j in range(n_per):
        cp_out(j).wait()


def build(cfg):
    @functools.partial(jax.jit, static_argnames=("A_seg_len",))
    def kernel_fn(A_x, A_mem0, A_Wq, A_Wk, A_Wv, A_Wo, A_seg_len, B_x, B_w1, B_b1, B_w2, B_b2):
        del B_x
        _, S, D = A_x.shape
        _, H, E = A_Wq.shape
        M = A_mem0.shape[1]
        seg = int(A_seg_len)
        n_seg = S // seg
        n_pro = cfg["n_pro"]
        hbm = pl.BlockSpec(memory_space=pl.ANY)
        vmem = pl.BlockSpec(memory_space=pltpu.VMEM)
        dma = pltpu.SemaphoreType.DMA
        wq, wk, wv = (w.reshape(D // 2, 2, H // 8, 8, E) for w in (A_Wq, A_Wk, A_Wv))
        out = pl.pallas_call(
            functools.partial(_kernel, d_ff=B_w1.shape[1], cfg=cfg),
            out_shape=jax.ShapeDtypeStruct((n_seg, seg, D), BF16),
            in_specs=[hbm, vmem, hbm, hbm, hbm, hbm, hbm, vmem, hbm, vmem],
            out_specs=hbm,
            scratch_shapes=[
                pltpu.VMEM((n_seg, seg, D), BF16),
                pltpu.VMEM((4 * n_pro, 8, D), BF16),
                pltpu.VMEM((len(QKV), 8 * n_pro, T), U32),
                pltpu.VMEM((M, D), F32),
                pltpu.VMEM((T, D), F32),
                pltpu.VMEM((T, D), F32),
                pltpu.VMEM((64 - M, D), F32),
                pltpu.VMEM((3 * H // 8 * D // 2, 8, E), U32),
                pltpu.VMEM((3, H // 8, 8, D // 2, E), U32),
                pltpu.VMEM((3, H // 8, len(SLOT), TP, T), U32),
                pltpu.VMEM((D // T, H // 4, 4, TP, T), U32),
                pltpu.VMEM((len(SLOT), 4, TP, T), U32),
                pltpu.VMEM((2, S // T, 7 * T, T), U32),
                pltpu.VMEM((len(QKV), 16, T), U32),
                pltpu.VMEM(((n_pro + 1) * 3 * H * 32, T), F32),
                pltpu.VMEM((32, H * E), F32),
                pltpu.VMEM((32, H * E), F32),
                dma((S // T + 1,)), dma((3 * H // 8,)), dma((4,)), dma((2,)), dma((S // T,)),
            ],
            compiler_params=pltpu.CompilerParams(vmem_limit_bytes=127 * 1024 * 1024,
                                                 **cfg.get("cp", {})),
            name="rmt_mixer",
        )(A_x.reshape(n_seg, seg, D), A_mem0.reshape(M, D), wq, wk, wv,
          A_Wo.reshape(H // 4, 4, E, D), B_w1.T, B_b1, B_w2, B_b2)
        return out.reshape(1, S, D)
    return kernel_fn


pallas_interleave_layers__memory_aug_recurrent_mem_tr__mixer_token_mlp__prompt_kernel = build(CFG)
```

```python
import functools
import math

import jax
import jax.numpy as jnp
from jax import lax
import jax.experimental.pallas as pl
import jax.experimental.pallas.tpu as pltpu

F32 = jnp.float32
BF16 = jnp.bfloat16
U32 = jnp.uint32
EPS = 1e-5
LOG2E = math.log2(math.e)
T = 128
TP = T // 2
R = 32
N_EARLY = 14

NN = (((1,), (0,)), ((), ()))
NT = (((1,), (1,)), ((), ()))

PLACEMENT = (
    dict(delay=((280, 150, 140, 170), (260, 240, 120, 170), (280, 170, 120, 170), (280, 240, 160, 150)),
         lag=(4, 2, 2, 2), singles=0, head_order=(1, 0, 2), out_last=7, out_group=4, mix_input_step=3),
    dict(delay=((260, 240, 140, 170), (260, 200, 140, 120), (260, 280, 140, 170), (280, 240, 140, 200)),
         lag=(2, 2, 2, 2), singles=2, head_order=(2, 1, 0), out_last=6, out_group=1, mix_input_step=2),
)
UP_ORDER = (5, 6, 1, 2, 0, 10, 7, 8, 9, 14, 13, 4, 3, 11, 12, 15, 16, 18, 19, 17, 21, 20,
            24, 23, 22, 32, 25, 27, 31, 26, 29, 30, 43, 36, 33, 28, 34, 37, 35, 39, 40, 38, 41, 42)
DOWN_ORDER = (1, 2, 3, 5, 4, 6, 0, 9, 8, 7, 10, 12, 11, 13, 14, 15, 16, 17, 18, 19, 20, 26,
              21, 28, 23, 24, 32, 22, 27, 29, 30, 34, 25, 31, 35, 33, 36, 37, 38, 39, 41, 42, 40, 43)


def _neg(a):
    return (-a[0], a[1])


def _add(a, b):
    if a is None:
        return b
    if a[0] == b[0]:
        return (a[0], a[1] + b[1])
    return (1, a[1] - b[1]) if a[0] > 0 else (1, b[1] - a[1])


def _sum(terms):
    return functools.reduce(_add, terms, None)


def _value(a):
    return a[1] if a[0] > 0 else -a[1]


def _terms(b, prod):
    kind, i, j = prod
    if kind < 3:
        return ((((1, i, 1), (1, j, 0)), ((1, i, 0), (1, j, 1))),
                (((1, i, 0), (-1, j, 0)), ((1, i, 0), (1, j, 0))),
                (((1, j, 1), (-1, i, 1)), ((1, i, 1), (1, j, 1))))[kind]
    h = int(i >= b)
    return ((((1, i, 0), (1, i, 1)), ((1, i, h),)),
            (((1, i, 1 - h),), ((1, i, 1 - h), (-1, i, h))))[kind - 3]


def _operand(b, prod, block):
    return _sum((s, block(v, h)) for s, v, h in _terms(b, prod)[0])


def _scatter(b, acc, results):
    update = {}
    for prod, sign, value in results:
        for s, v, h in _terms(b, prod)[1]:
            update[v, h] = _add(update.get((v, h)), (s * sign, value))
    for key, term in update.items():
        acc[key] = _add(acc.get(key), term)


def _folded_inputs(b, block):
    return lambda v, h: block(v, h) if v < b else block(b, h) + block(v - b, h)


def _folded_output(acc, b, n, h):
    if n < b:
        return _add(acc[n, h], _neg(acc[b + n, h]))
    return _sum(acc[b + j, h] for j in range(b))


def _weights(b, fold_inputs, tile, share_tiles=False):
    links = {}

    def make_link(u, v):
        m, n = u % b, v % b
        others = [k for k in range(b) if k != m]
        if m != n:
            if fold_inputs:
                return (1, tile(m, v))
            return (1 if u >= b else -1, tile(u, n))
        if fold_inputs:
            if u >= b:
                return (1, tile(b, v)) if v >= b else _sum(
                    [(1, tile(b, m))] + [(-1, tile(k, m)) for k in others])
            if v >= b:
                return _add((1, tile(m, v)), (-1, tile(b, v)))
            return _add((1, tile(m, m)), _neg(link(b + m, m)))
        if u >= b:
            return (1, tile(u, b)) if v >= b else _add((1, tile(u, m)), (1, tile(u, b)))
        if v >= b:
            return _sum([(1, tile(m, b))] + [(1, tile(m, k)) for k in others])
        return _add((1, tile(m, m)), link(m, b + m))

    def link(u, v):
        if (u, v) not in links or (u % b != v % b and not share_tiles):
            links[u, v] = make_link(u, v)
        return links[u, v]

    def weight(prod):
        kind, i, j = prod
        if kind == 0:
            return _add(link(i, j), link(j, i))
        if kind < 3:
            return link(i, j) if kind == 1 else link(j, i)
        across = range(b) if i >= b else range(b, 2 * b)
        if kind == 3:
            if fold_inputs:
                return _sum([link(i, i)] + [_neg(link(i, w)) for w in across])
            if i < b:
                return _add(link(i, i), (-1, tile(i, b)))
            return _sum((-1, tile(i, k)) for k in range(b))
        if not fold_inputs:
            return _sum([link(i, i)] + [link(w, i) for w in across])
        if i < b:
            return _add(link(i, i), (1, tile(b, i)))
        return _sum((1, tile(k, i)) for k in range(b))
    return weight


def _is_plain(b, prod):
    kind, i, j = prod
    return kind in (1, 2) and i != j - b


def _edge(i, j):
    return [(kind, i, j) for kind in range(3)]


def _corners(v):
    return [(3, v, v), (4, v, v)]


def _products_by_diagonal(b):
    first = [(1, i, j) for i in range(2) for j in (2 * b - 2, 2 * b - 1)]
    prods = []
    for m in range(b):
        prods += [p for j in range(b) if j != m for p in _edge(m, b + j)]
        prods += _edge(m, b + m) + _corners(m) + _corners(b + m)
    return first + [p for p in prods if p not in first]


def _products_nested(b):
    prods = []
    for m in range(b):
        prods += [(kind, m, b + j) for kind in range(3) for j in range(m)] + _corners(m)
        prods += [(kind, i, b + m) for kind in range(3) for i in range(m + 1)] + _corners(b + m)
    return prods


def _products_grouped(fold_inputs):
    b = 7
    corners = {v: _corners(v)[::-1 if fold_inputs else 1] for v in range(2 * b)}

    def square(i, j):
        return [[(kind, i + x, b + j + y) for x in range(2) for y in range(2)] for kind in range(3)]

    def singles(spec):
        return [_edge(int(i), b + int(j)) + [corners[int(i) if side == "L" else b + int(j)].pop(0)]
                for i, j, side in spec.split()]

    light = square(1, 3) + square(3, 1) + square(1, 5) + square(5, 1) + square(3, 5)
    heavy = singles("03L 10L 01R 20L 02R 30R 40R 04R 50L 05R 60L 06R 00L 12R 21R 11L 22L")
    groups = [g for pair in zip(light, heavy) for g in pair] + heavy[len(light):]
    groups += singles("34L 53R 63R 43L 33L 54R 64L 44L 56R 65R 55L") + [_edge(6, b + 6)]
    return [groups[n] for n in (UP_ORDER if fold_inputs else DOWN_ORDER)]


QKV_PRODUCTS = _products_by_diagonal(4)
OUT_PRODUCTS = _products_nested(4)
SLOT = {p: n for n, p in enumerate(p for p in QKV_PRODUCTS if not _is_plain(4, p))}


def _dot(a, b, dims=NN):
    return lax.dot_general(a, b, dims, preferred_element_type=F32)


def _layernorm(x):
    inv_d = 1.0 / x.shape[-1]
    c = x - jnp.sum(x, axis=-1, keepdims=True) * inv_d
    var = jnp.sum(c * c, axis=-1, keepdims=True) * inv_d
    return c * lax.rsqrt(var + EPS)


def _gelu(x):
    k = math.sqrt(2.0 / math.pi)
    inner = x * (k + (k * 0.044715) * (x * x))
    half = 0.5 * x
    return half + half * jnp.tanh(inner)


def _as_bf16(words):
    return pltpu.bitcast(words, BF16)


def _as_words(x):
    return pltpu.bitcast(x.astype(BF16), U32)


def _split_rows(words):
    return jnp.concatenate([pltpu.bitcast(words << 16, F32),
                            pltpu.bitcast(words & jnp.uint32(0xFFFF0000), F32)], axis=0)


def _join_rows(x):
    x = pltpu.bitcast(x.astype(BF16).astype(F32), U32)
    n = x.shape[0] // 2
    return (x[0:n] >> 16) | x[n:]


def _rows(start, size, align):
    if isinstance(start, int):
        return pl.ds(start, size)
    return pl.ds(pl.multiple_of(start, align), size)


def _kernel(x_hbm, mem0_hbm, wq_hbm, wk_hbm, wv_hbm, wo_hbm, w1t_hbm, b1_hbm, w2_hbm, b2_hbm,
            out_hbm,
            raw, wqkv, wqkv_sum, wo, wo_sum, act, early_lhs, lhs, o_main, o_spare, x,
            delta, normed, first, mem, x_early, mem0, b1, b2,
            x_sem, w_sem, wo_sem, mix_sem, small_sem, out_sem):
    n_seg, seg, D = x.shape
    S = n_seg * seg
    M = mem0.shape[0]
    L = M + seg
    X = L - R
    P = R // X
    n_per = n_seg // P
    H, E = wqkv.shape[1] * wqkv.shape[2], wqkv.shape[4]
    KT = D // T
    d_ff = b1.shape[0]
    assert (KT, E, X, P * seg, n_per, H) == (5, T, 8, T, 16, 32)
    assert 13 * T < d_ff < 14 * T and d_ff % 16 == 0 and N_EARLY == n_per - 2

    def spare_rows(j, i, h, r0=0, rn=R):
        return _rows((((j + 1) * 3 + i) * H + h) * R + r0, rn, X)

    def mix_rows(j, r0, rn):
        return _rows(j * 2 * D + r0, rn, X)

    def resid_rows(j, k, r0, rn):
        return _rows(j * 2 * D + D + k * T + r0, rn, X)

    def hidden_rows(f, h):
        return pl.ds(n_per * 2 * D + (2 * f + h) * (D // 2), D // 2)

    def out_block(v):
        return 2 * (v % 4) + v // 4

    staged = raw.reshape(raw.shape[0] * 8, E)

    def mix_weight_rows(i, t, r0, rn):
        return _rows((i * n_per + t) * 14 * TP + r0, rn, X)

    cp_early = pltpu.make_async_copy(x_hbm.at[0:N_EARLY * P, R - M:seg, :], x_early, x_sem.at[n_per])
    cp_small = [pltpu.make_async_copy(src, dst, small_sem.at[n])
                for n, (src, dst) in enumerate(((mem0_hbm, mem0), (b1_hbm, b1), (b2_hbm, b2)))]
    cp_mix = [pltpu.make_async_copy(w.bitcast(U32).at[:, t * T:(t + 1) * T],
                                    staged.at[mix_weight_rows(i, t, 0, d_ff // 2), :], mix_sem)
              for i, w in enumerate((w1t_hbm, w2_hbm)) for t in range(S // T)]

    def cp_x(j):
        segs = pl.ds(j * P, P)
        return pltpu.make_async_copy(x_hbm.at[segs], x.at[segs], x_sem.at[j])

    def cp_out(j):
        segs = pl.ds(j * P, P)
        return pltpu.make_async_copy(x.at[segs], out_hbm.at[segs], out_sem)

    def cp_w(w, c, g):
        return [pltpu.make_async_copy(w.bitcast(U32).at[:, p, g],
                                      raw.at[pl.ds(c * (D // 2), D // 2), pl.ds(4 * p, 4), :], w_sem.at[c])
                for p in range(2)]

    def cp_wo(q):
        return [pltpu.make_async_copy(wo_hbm.bitcast(U32).at[:, q, :, n * T:(n + 1) * T],
                                      wo.at[n, :, q], wo_sem.at[q]) for n in range(KT)]

    def start_chunk(c, g, i):
        for n, w in enumerate((wq_hbm, wk_hbm, wv_hbm)):
            @pl.when(i == n)
            def _():
                for cp in cp_w(w, c, g):
                    cp.start()

        @pl.when((c >= 3) & (c % 2 == 1) & (c <= 9))
        def _():
            for cp in cp_wo((c - 3) // 2):
                cp.start()

    cp_early.start()
    lax.fori_loop(0, 3, lambda c, _: start_chunk(c, 0, c), None)
    cp_early.wait()
    xn = _layernorm(x_early[...].astype(F32).reshape(N_EARLY * R, D))
    n_half = N_EARLY * R // 2
    early_block = _folded_inputs(4, lambda k, h: xn[h * n_half:(h + 1) * n_half, k * T:(k + 1) * T])
    lhs_sign, qkv_sign, out_sign = {}, {}, {}
    for r, prod in enumerate(QKV_PRODUCTS):
        lhs_sign[prod], v = _operand(4, prod, early_block)
        early_lhs[r] = _as_words(v)

    def prologue(c, _, with_wo):
        g = c // 3
        i = c - 3 * g

        @pl.when(g < 3)
        def _():
            start_chunk(c + 3, g + 1, i)

        @pl.when(c == 10)
        def _():
            for cp in [cp_x(0), cp_x(1)] + cp_small:
                cp.start()

        for cp in cp_w(wq_hbm, c, 0):
            cp.wait()
        pending = []
        if with_wo:
            quarter = (c - 4) // 2
            part = _rows((c % 2) * (TP // 2), TP // 2, TP // 2)

            @pl.when(c % 2 == 0)
            def _():
                for cp in cp_wo(quarter):
                    cp.wait()
            out_weight = _weights(4, False, lambda v, n: _split_rows(wo[n, out_block(v), quarter, part, :]))
            pending = list(SLOT)
        done = set()

        def words(k, h):
            if (k, h // 2) not in done:
                done.add((k, h // 2))
                row = (c * (D // 2) + k * TP) * 8 + h // 2
                even, odd = [staged[pl.ds(row + 4 * p, TP, stride=8), :] for p in range(2)]
                h0 = h // 2 * 2
                wqkv[i, g, h0, k * TP:(k + 1) * TP, :] = (even & jnp.uint32(0xFFFF)) | (odd << 16)
                wqkv[i, g, h0 + 1, k * TP:(k + 1) * TP, :] = (even >> 16) | (odd & jnp.uint32(0xFFFF0000))
            return wqkv[i, g, h, k * TP:(k + 1) * TP, :]

        plain = _weights(4, True, words)
        summed = _weights(4, True, lambda k, h: _split_rows(words(k, h)))
        acc, group = {}, []
        for r, prod in enumerate(QKV_PRODUCTS):
            if prod in SLOT:
                s, w = summed(prod)
                w = _join_rows(w)
                wqkv_sum[i, g, SLOT[prod]] = w
            else:
                s, w = plain(prod)
            qkv_sign[prod] = lhs_sign[prod] * s
            if pending and (len(SLOT) - len(pending)) * 7 <= (r - 8) * 5:
                other = pending.pop(0)
                out_sign[other], piece = out_weight(other)
                piece = _join_rows(piece)
                wo_sum[SLOT[other], quarter, part, :] = piece
                w = jnp.concatenate([jnp.where(c < 0, piece, w[0:TP // 2]), w[TP // 2:]], axis=0)
            group.append((prod, qkv_sign[prod], _dot(_as_bf16(early_lhs[r]), _as_bf16(w))))
            if len(group) == 4:
                _scatter(4, acc, group)
                group = []
        assert not pending
        for h in range(8):
            for half in range(2):
                v = _value(acc[h, half])
                for p in range(N_EARLY // 2):
                    act[spare_rows(half * (N_EARLY // 2) + p, i, 8 * g + h), :] = v[p * R:(p + 1) * R]

    lax.fori_loop(0, 4, functools.partial(prologue, with_wo=False), None)
    lax.fori_loop(4, 12, functools.partial(prologue, with_wo=True), None)
    n_pad = 14 * TP - d_ff // 2
    for t in range(2 * n_per):
        staged[mix_weight_rows(0, t, d_ff // 2, n_pad), :] = jnp.zeros((n_pad, T), U32)
    for cp in [cp_x(0)] + cp_small:
        cp.wait()


    def residual(j):
        for u in range(P):
            v = x[j * P + u].astype(F32) + delta[u * seg:(u + 1) * seg, :]
            for k in range(KT):
                act[resid_rows(j, k, u * seg, seg), :] = v[:, k * T:(k + 1) * T]

    def mix_input(j):
        for r in range(0, T, 16):
            v = jnp.concatenate([act[resid_rows(j, k, r, 16), :] for k in range(KT)], axis=1)
            normed[r:r + 16, :] = _layernorm(_layernorm(v))
        for k in range(KT):
            act[mix_rows(j, k * T, T), :] = normed[:, k * T:(k + 1) * T].T

    def first_rows(j):
        first[0:R - M, :] = _layernorm(x[j * P].astype(F32)[0:R - M])
        for u in range(P):
            first[R - M + u * X:R - M + (u + 1) * X, :] = _layernorm(x[j * P + u].astype(F32)[R - M:seg])

    def begin_layer():
        mem[...] = mem0[...].astype(F32)
        delta[...] = jnp.zeros(delta.shape, F32)
        first_rows(0)

    def step(u, rows, spare, slot, tune):
        last = u == P - 1
        query = lax.broadcasted_iota(jnp.int32, (L, T), 0)
        lane = lax.broadcasted_iota(jnp.int32, (1, T), 1)
        key = lane - jnp.where(lane >= 2 * L, 2 * L, jnp.where(lane >= L, L, 0))
        mask = jnp.where(query < M, L - 1, query) >= key
        fill = jnp.where(lane < 3 * L, -1e9 * LOG2E, -jnp.inf)
        groups = [(lane >= c * L) & (lane < (c + 1) * L) for c in range(3)]
        clock = [0]
        qkv, state, has_k, has_v, has_o = {}, {}, {}, {}, {}

        def full(h, i):
            return jnp.concatenate([qkv[h, i], act[spare_rows(slot, i, h, u * X, X), :]], axis=0)

        n1 = tune["singles"]
        units = ([(h,) for h in range(n1)] + [(h, h + 1, h + 2) for h in range(n1, n1 + 30, 3)]
                 + [(h,) for h in range(n1 + 30, H)])
        triples = [n for n, unit in enumerate(units) if len(unit) == 3]
        partner = {n: triples[i - tune["lag"][u]] for i, n in enumerate(triples) if i >= tune["lag"][u]}
        keys, done = {}, {}

        def own(c, inside, outside):
            return jnp.where(groups[c], inside, outside)

        def by_lane(parts):
            return functools.reduce(lambda out, c: own(c, parts[c], out), range(len(parts) - 1), parts[-1])

        def stacked(parts):
            return jnp.concatenate(list(parts) + [jnp.zeros((T - 3 * L, E), F32)], axis=0)

        def flip_keys(n):
            keys[n] = stacked(full(h, 1) for h in units[n]).T

        def scores(n):
            if len(units[n]) == 1:
                h = units[n][0]
                state[n] = _dot(full(h, 0), full(h, 1).astype(BF16), NT)
            else:
                k = keys[n].astype(BF16)
                state[n] = by_lane([_dot(full(h, 0), k) for h in units[n]])

        def row_max(n):
            w = state[n].shape[1]
            t = jnp.where(mask[:, 0:w], state[n] * (float(E) ** -0.5 * LOG2E), fill[:, 0:w])
            if len(units[n]) == 1:
                state[n] = t - jnp.max(t, axis=-1, keepdims=True)
            else:
                state[n] = t - by_lane(
                    [jnp.max(own(c, t, -jnp.inf), axis=-1, keepdims=True) for c in range(3)])

        def row_sum(n):
            e = jnp.exp2(state[n])
            if len(units[n]) == 1:
                total = jnp.sum(e, axis=-1, keepdims=True)
            else:
                total = by_lane([jnp.sum(own(c, e, 0.0), axis=-1, keepdims=True) for c in range(3)])
            inv = pl.reciprocal(total, approx=True)
            state[n] = e * (inv * (2.0 - total * inv))

        def keep(h, o):
            if last:
                o_main[:, h * E:(h + 1) * E] = o[0:R]
            else:
                o_main[0:R // 2, h * E:(h + 1) * E] = pltpu.bitcast(_as_words(o[0:R]), F32)
            o_spare[u * X:(u + 1) * X, h * E:(h + 1) * E] = o[R:L]
            has_o[h] = clock[0]

        def values(n):
            if len(units[n]) == 1:
                keep(units[n][0], _dot(state[n], full(units[n][0], 2).astype(BF16)))
                return
            v = stacked(full(h, 2) for h in units[n]).astype(BF16)
            for c, h in enumerate(units[n]):
                keep(h, _dot(own(c, state[n], 0.0), v))

        def scores_and_values(n, m):
            p = state[m]
            q = [full(h, 0) for h in units[n]]
            v = [full(h, 2) for h in units[m]]
            k = [own(c, keys[n], 0.0) for c in range(3)]
            both = []
            for c in range(3):
                w = ([k[c][0:c * L]] if c else []) + [own(c, 0.0, v[c]), k[c][(c + 1) * L:]]
                both.append(_dot(own(c, p, q[c]), jnp.concatenate(w, axis=0).astype(BF16)))
            rest_s = _dot(by_lane(q), stacked(k[c][c * L:(c + 1) * L] for c in range(3)).astype(BF16))
            rest_o = _dot(p, stacked(own(c, v[c], 0.0) for c in range(3)).astype(BF16))
            state[n] = rest_s + by_lane(both)
            for c, h in enumerate(units[m]):
                keep(h, own(c, rest_o, both[c]))

        delay = tune["delay"][u]
        todo = [(stage, n) for n in range(len(units)) for stage in range(5)
                if (stage != 0 or n in triples) and (stage != 4 or n not in partner.values())]

        def due(stage, n):
            def after(times, items, wait):
                return max(times[i] for i in items) + wait if all(i in times for i in items) else None

            def values_due(m):
                return [after(done, [(3, m)], delay[3]), after(has_v, units[m], delay[0])]
            if stage == 0 or (stage == 1 and n not in triples):
                times = [after(has_k, units[n], delay[0])]
            elif stage == 1:
                times = [after(done, [(0, n)], 150)] + (values_due(partner[n]) if n in partner else [])
            elif stage < 4:
                times = [after(done, [(stage - 1, n)], delay[stage - 1])]
            else:
                times = values_due(n)
            return None if None in times else max(times)

        def advance(tiles, force=False):
            clock[0] += tiles * R // 4
            while True:
                ready = [(t, task) for task in todo if (t := due(*task)) is not None]
                if not ready or (min(ready)[0] > clock[0] and not force):
                    return
                stage, n = min(ready)[1]
                todo.remove((stage, n))
                if stage == 1 and n in partner:
                    clock[0] += 5 * L // 4
                    scores_and_values(n, partner[n])
                else:
                    clock[0] += len(units[n]) * L // 4 if stage in (1, 4) else 0
                    (flip_keys, scores, row_max, row_sum, values)[stage](n)
                done[stage, n] = clock[0]
                force = False

        def need(h):
            while any(g not in has_o for g in range(h + 1)):
                advance(0, force=True)

        if spare is not None:
            block = _folded_inputs(4, lambda k, h: (rows, spare)[h][:, k * T:(k + 1) * T])
            for r, prod in enumerate(QKV_PRODUCTS):
                lhs[r] = _as_words(_operand(4, prod, block)[1])
            for g in range(H // 8):
                for i in range(3):
                    plain = _weights(4, True, lambda k, h: wqkv[i, g, h, k * TP:(k + 1) * TP, :])
                    acc, group = {}, []
                    for r, prod in enumerate(QKV_PRODUCTS):
                        w = wqkv_sum[i, g, SLOT[prod]] if prod in SLOT else plain(prod)[1]
                        group.append((prod, qkv_sign[prod], _dot(_as_bf16(lhs[r]), _as_bf16(w))))
                        if len(group) == 2:
                            _scatter(4, acc, group)
                            group = []
                        advance(1)
                    for h in range(8):
                        qkv[8 * g + h, i] = _value(acc[h, 0])
                        act[spare_rows(slot, i, 8 * g + h), :] = _value(acc[h, 1])
                        if i > 0:
                            (has_k, has_v)[i - 1][8 * g + h] = clock[0]
        else:
            rows = rows.astype(BF16)
            lead = 2
            for k in range(KT):
                for h in range(lead):
                    for i in range(3):
                        r = _dot(rows[:, k * T:(k + 1) * T], _as_bf16(wqkv[i, 0, h, k * TP:(k + 1) * TP, :]))
                        qkv[h, i] = r if k == 0 else qkv[h, i] + r
            advance(3 * lead * KT)
            for h in range(lead):
                has_k[h] = has_v[h] = clock[0]
            for h in range(lead, H):
                for i in tune["head_order"]:
                    qkv[h, i] = _dot(rows, _as_bf16(wqkv[i, h // 8, h % 8]))
                    if i > 0:
                        (has_k, has_v)[i - 1][h] = clock[0] + KT * R // 4
                    advance(KT)

        if last:
            acc = {}
            plain = _weights(4, False, lambda v, n: wo[n, out_block(v)])
            group = []
            for prod in OUT_PRODUCTS:
                need(max(out_block(v) for v in prod[1:]) * 4 + 3)
                s, v = _operand(4, prod, lambda v, h: (o_main, o_spare)[h][
                    :, out_block(v) * 4 * E:(out_block(v) + 1) * 4 * E])
                sw, w = (out_sign[prod], wo_sum[SLOT[prod]]) if prod in SLOT else plain(prod)
                group.append((prod, s * sw, _dot(v, _as_bf16(w.reshape(4 * TP, T)))))
                if len(group) == tune["out_group"]:
                    _scatter(4, acc, group)
                    group = []
                advance(4)
            o, rest = [jnp.concatenate([_value(_folded_output(acc, 4, n, h)) for n in range(KT)], axis=1)
                       for h in range(2)]
            for p in range(P):
                delta[p * seg + R - M:(p + 1) * seg, :] = rest[p * X:(p + 1) * X]
        else:
            acc = [None] * KT
            tail = H - tune["out_last"]
            bounds = list(range(tail)) + [tail, H]
            for h0, h1 in zip(bounds[:-1], bounds[1:]):
                need(h1 - 1)
                a = _as_bf16(o_main[0:R // 2, h0 * E:h1 * E])
                for n in range(KT):
                    w = jnp.concatenate([wo[n, h // 4, h % 4] for h in range(h0, h1)], axis=0)
                    r = _dot(a, _as_bf16(w))
                    acc[n] = r if acc[n] is None else acc[n] + r
                    advance(h1 - h0)
            o = jnp.concatenate(acc, axis=1)
        delta[u * seg:u * seg + R - M, :] = o[M:R]
        return o[0:M]

    def period(j, _, early):
        tune = PLACEMENT[early]
        if early:
            cp_x(j + 1).wait()
            cp_x(j + 2).start()
            for i in range(4):
                @pl.when(j == i)
                def _():
                    for cp in cp_mix[8 * i:8 * i + 8]:
                        cp.start()
        prev = jnp.maximum(j - 1, 0)
        head_rows = first[...]
        memory = mem[...]
        residual(prev)
        for u in range(P):
            if u == tune["mix_input_step"]:
                mix_input(prev)
            if u == P - 1:
                first_rows(jnp.minimum(j + 1, n_per - 1))
            tokens = head_rows[0:R - M] if u == 0 else _layernorm(x[j * P + u].astype(F32)[0:R - M])
            memory = step(u, jnp.concatenate([memory, tokens], axis=0),
                          head_rows[R - M:] if u == 0 and not early else None,
                          j if early else N_EARLY - 1, tune)
        mem[...] = memory

    def token_mix(li):
        half = D // 2
        bias1 = jnp.concatenate(
            [b1[...].astype(F32).reshape(1, d_ff), jnp.zeros((1, 14 * T - d_ff), F32)], axis=1)
        bias2 = b2[...].astype(F32).reshape(1, S)

        def matmul(fold_inputs, operand, tile, dims, finish):
            plain = _weights(7, fold_inputs, tile)
            summed = _weights(7, fold_inputs, lambda u, v: tile(u, v).astype(F32), share_tiles=True)
            groups = _products_grouped(fold_inputs)
            acc = {}
            for n, group in enumerate(groups):
                results = []
                for prod in group:
                    s, v = operand(prod)
                    sw, w = (plain if _is_plain(7, prod) else summed)(prod)
                    results.append((prod, s * sw, _dot(v, w, dims)))
                _scatter(7, acc, results)
                later = {v % 7 for rest in groups[n + 1:] for prod in rest for v in prod[1:]}
                for m in sorted({v % 7 for prod in group for v in prod[1:]} - later):
                    finish(acc, m)
            return acc

        def tile(i, f, t):
            return _as_bf16(staged[mix_weight_rows(i, t, f * TP, TP), :])

        def token_tile(n, t):
            return (2 * n + 2) % n_per + t

        tokens = _folded_inputs(7, lambda n, h: jnp.concatenate(
            [act[mix_rows(token_tile(n, t), h * half, half), :] for t in range(2)], axis=1))
        waiting, count = [], [0]

        def activate(acc, f, h):
            g = _gelu(_value(_add(acc[f, h], (1, bias1[:, f * T:(f + 1) * T]))))
            act[hidden_rows(f, h), :] = g
            return g

        def schedule(acc, m):
            for f in (m, 7 + m):
                for h in range(2):
                    when = max(count[0] + 5, waiting[-1][0] + 2 if waiting else 0)
                    waiting.append((when, functools.partial(activate, acc, f, h)))

        def up_operand(prod):
            s, v = _operand(7, prod, tokens)
            count[0] += 1
            if waiting and waiting[0][0] <= count[0]:
                v = jnp.concatenate([jnp.where(li > 2, waiting.pop(0)[1](), v[:, 0:T]), v[:, T:]], axis=1)
            return s, v

        matmul(True, up_operand,
               lambda n, f: jnp.concatenate([tile(0, f, token_tile(n, t)) for t in range(2)], axis=1),
               NT, schedule)
        for _, task in waiting:
            task()

        def down(t, _):
            def down_operand(prod):
                s, v = _operand(7, prod, lambda f, h: act[hidden_rows(f, h), :])
                return s, v.astype(BF16)

            def emit(acc, n):
                j = 2 * n + t
                bias = jnp.where(t == 0, bias2[:, 2 * n * T:(2 * n + 1) * T],
                                 bias2[:, (2 * n + 1) * T:(2 * n + 2) * T])
                y = jnp.concatenate(
                    [_value(_add(_folded_output(acc, 7, n, h), (1, bias))) for h in range(2)], axis=0)
                v = jnp.concatenate([act[resid_rows(j, k, 0, T), :] for k in range(KT)], axis=1) + y.T
                x[pl.ds(j * P, P)] = v.reshape(P, seg, D).astype(BF16)
                cp_out(j).start()
                if n == 0:
                    begin_layer()
            emit(matmul(False, down_operand, lambda f, n: tile(1, f, 2 * n + t), NN, emit), 7)
        lax.fori_loop(0, 2, down, None)

    begin_layer()
    lax.fori_loop(0, N_EARLY, functools.partial(period, early=True), None)
    for cp in [cp_x(n_per - 1)] + cp_mix:
        cp.wait()

    def layer(li, _):
        lax.fori_loop(jnp.where(li == 0, N_EARLY, 0), n_per, functools.partial(period, early=False), None)

        @pl.when(li > 0)
        def _():
            pltpu.make_async_copy(x, out_hbm, out_sem).wait()
        residual(n_per - 1)
        mix_input(n_per - 1)
        token_mix(li)

    lax.fori_loop(0, 2, layer, None)
    pltpu.make_async_copy(x, out_hbm, out_sem).wait()


@functools.partial(jax.jit, static_argnames=("A_seg_len",))
def pallas_interleave_layers__memory_aug_recurrent_mem_tr__mixer_token_mlp__prompt_kernel(
    A_x, A_mem0, A_Wq, A_Wk, A_Wv, A_Wo, A_seg_len, B_x, B_w1, B_b1, B_w2, B_b2,
):
    del B_x
    _, S, D = A_x.shape
    _, H, E = A_Wq.shape
    M = A_mem0.shape[1]
    seg = A_seg_len
    n_seg = S // seg
    hbm = pl.BlockSpec(memory_space=pl.ANY)
    vmem = pltpu.VMEM
    dma = pltpu.SemaphoreType.DMA
    wq, wk, wv = (w.reshape(D // 2, 2, H // 8, 8, E) for w in (A_Wq, A_Wk, A_Wv))
    out = pl.pallas_call(
        _kernel,
        out_shape=jax.ShapeDtypeStruct((n_seg, seg, D), BF16),
        in_specs=[hbm] * 10,
        out_specs=hbm,
        scratch_shapes=[
            vmem((3 * H // 8 * D // 2 + 4, 8, E), U32),
            vmem((3, H // 8, 8, D // 2, E), U32),
            vmem((3, H // 8, len(SLOT), TP, T), U32),
            vmem((D // T, H // 4, 4, TP, T), U32),
            vmem((len(SLOT), 4, TP, T), U32),
            vmem(((N_EARLY + 1) * 3 * H * R, T), F32),
            vmem((len(QKV_PRODUCTS), N_EARLY * R // 4, T), U32),
            vmem((len(QKV_PRODUCTS), R // 2, T), U32),
            vmem((R, H * E), F32),
            vmem((R, H * E), F32),
            vmem((n_seg, seg, D), BF16),
            vmem((T, D), F32),
            vmem((T, D), F32),
            vmem((2 * R - M, D), F32),
            vmem((M, D), F32),
            vmem((4 * N_EARLY, 8, D), BF16),
            vmem((M, D), BF16),
            vmem(B_b1.shape, BF16),
            vmem(B_b2.shape, BF16),
            dma((S // T + 1,)), dma((3 * H // 8,)), dma((4,)), dma(()), dma((3,)), dma(()),
        ],
        compiler_params=pltpu.CompilerParams(vmem_limit_bytes=127 * 1024 * 1024,
                                             disable_bounds_checks=True),
        name="rmt_mixer",
    )(A_x.reshape(n_seg, seg, D), A_mem0.reshape(M, D), wq, wk, wv,
      A_Wo.reshape(H // 4, 4, E, D), B_w1.T, B_b1, B_w2, B_b2)
    return out.reshape(1, S, D)
```
